```python
import os as _os
_os.environ.setdefault("JAX_PLATFORMS", "cpu")
import jax
import jax.numpy as jnp

def _softmax(x, axis=-1):
    return jax.nn.softmax(x, axis=axis)
def _gelu(x):
    return jax.nn.gelu(x, approximate=True)
def _silu(x):
    return jax.nn.silu(x)
def _sigmoid(x):
    return jax.nn.sigmoid(x)
def _layernorm(x, axis=-1, eps=1e-5):
    m = jnp.mean(x, axis=axis, keepdims=True)
    v = jnp.var(x, axis=axis, keepdims=True)
    return (x - m) / jnp.sqrt(v + eps)
def _scatter_add(tgt, idx, src, axis=0):
    return tgt.at[idx].add(src)
def _segment_sum(src, seg, n):
    return jax.ops.segment_sum(src, seg, n)
class _Rng:
    def __init__(self, key):
        self._k = key
    def _next(self):
        self._k, sub = jax.random.split(self._k)
        return sub
    def normal(self, shape):
        return jax.random.normal(self._next(), shape, dtype=jnp.bfloat16)
    def randint(self, lo, hi, shape):
        return jax.random.randint(self._next(), shape, lo, hi, dtype=jnp.int32)
    def uniform(self, shape, lo=0.0, hi=1.0):
        return jax.random.uniform(self._next(), shape, jnp.bfloat16, lo, hi)
    def permutation(self, n):
        return jax.random.permutation(self._next(), n)


kernel_name = 'standalone__mha_softmax__near_ridge'

def setup_inputs():
    _rng = _Rng(jax.random.key(int.from_bytes(__import__("os").urandom(4), "little")))
    _w = (lambda a: (lambda t: t.astype(jnp.bfloat16) if jnp.issubdtype(t.dtype, jnp.floating) else t)(jnp.asarray(a)))
    B, H, Sq, Sk, D = 16, 16, 256, 256, 256
    return {
        "q": _w((lambda *s: _rng.normal(s) * 0.4)(B, H, Sq, D)),
        "k": _w((lambda *s: _rng.normal(s) * 0.4)(B, H, Sk, D)),
        "v": _w((lambda *s: _rng.normal(s) * 0.05)(B, H, Sk, D)),
    }

def reference(q, k, v):
    scale = q.shape[-1] ** -0.5
    scores = jnp.einsum("bhqd,bhkd->bhqk", q, k) * scale
    p = _softmax(scores, axis=-1)
    return jnp.einsum("bhqk,bhkd->bhqd", p, v)
```

```python
import math

import jax
import jax.numpy as jnp
import jax.experimental.pallas as pl
import jax.experimental.pallas.tpu as pltpu

_LOG2E = math.log2(math.e)


def _attend(q, k, v, scale):
    s = jax.lax.dot_general(
        q, k, (((1,), (1,)), ((), ())), preferred_element_type=jnp.float32
    )
    m = jnp.max(s, axis=-1, keepdims=True)
    p = jnp.exp2((s - m) * (scale * _LOG2E))
    l = jnp.sum(p, axis=-1, keepdims=True)
    o = jnp.dot(p.astype(v.dtype), v, preferred_element_type=jnp.float32)
    return o * (1.0 / l)


@jax.jit
def pallas_standalone__mha_softmax__near_ridge_kernel(
    q: jax.Array,
    k: jax.Array,
    v: jax.Array,
):
    B, H, Sq, D = q.shape
    Sk = k.shape[2]
    N = B * H
    scale = D ** -0.5

    c = 4
    R = 4
    n = N // c
    wrows = 128
    Rw = 32
    G = 16
    rows = N * Sq
    nw = rows // wrows
    assert N % c == 0 and n >= R and rows % wrows == 0 and nw % G == 0 and nw >= Rw

    def kernel_function(q_h, k_h, v_h, o_h, qb, kb, vb, ob, rsem, wsem):
        srcs = (q_h, k_h, v_h)
        bufs = (qb, kb, vb)

        def rd(s, i, slot):
            return pltpu.make_async_copy(
                srcs[s].at[pl.ds(i * c, c)], bufs[s].at[slot], rsem.at[s, slot]
            )

        def wr(i, slot):
            j = (i % G) * (nw // G) + i // G
            r = pl.multiple_of(j * wrows, wrows)
            return pltpu.make_async_copy(
                ob.at[pl.ds(r, wrows)], o_h.at[pl.ds(r, wrows)], wsem.at[slot]
            )

        for i in range(R):
            for s in range(3):
                rd(s, i, i).start()

        def read_body(i, carry):
            slot = i % R

            @pl.when(i == n - 1)
            def _():
                def issue(t, carry):
                    wr(t, t).start()
                    return carry

                jax.lax.fori_loop(0, Rw, issue, None)

            for s in range(3):
                rd(s, i, slot).wait()
            for u in range(c):
                r = pl.multiple_of((i * c + u) * Sq, Sq)
                ob[pl.ds(r, Sq), :] = _attend(
                    qb[slot, u], kb[slot, u], vb[slot, u], scale
                ).astype(ob.dtype)

            @pl.when(i + R < n)
            def _():
                for s in range(3):
                    rd(s, i + R, slot).start()

            return carry

        jax.lax.fori_loop(0, n, read_body, None)

        def write_body(i, carry):
            slot = i % Rw
            wr(i, slot).wait()

            @pl.when(i + Rw < nw)
            def _():
                wr(i + Rw, slot).start()

            return carry

        jax.lax.fori_loop(0, nw, write_body, None)

    out = pl.pallas_call(
        kernel_function,
        in_specs=[pl.BlockSpec(memory_space=pl.ANY)] * 3,
        out_specs=pl.BlockSpec(memory_space=pl.ANY),
        out_shape=jax.ShapeDtypeStruct((rows, D), v.dtype),
        scratch_shapes=[
            pltpu.VMEM((R, c, Sq, D), q.dtype),
            pltpu.VMEM((R, c, Sk, D), k.dtype),
            pltpu.VMEM((R, c, Sk, D), v.dtype),
            pltpu.VMEM((rows, D), v.dtype),
            pltpu.SemaphoreType.DMA((3, R)),
            pltpu.SemaphoreType.DMA((Rw,)),
        ],
        compiler_params=pltpu.CompilerParams(vmem_limit_bytes=64 * 1024 * 1024),
    )(q.reshape(N, Sq, D), k.reshape(N, Sk, D), v.reshape(N, Sk, D))
    return out.reshape(B, H, Sq, D)
```

```python
import math

import jax
import jax.numpy as jnp
import jax.experimental.pallas as pl
import jax.experimental.pallas.tpu as pltpu

_LOG2E = math.log2(math.e)


def _attend(q, k, v, scale):
    s = jax.lax.dot_general(
        q, k, (((1,), (1,)), ((), ())), preferred_element_type=jnp.float32
    )
    m = jnp.max(s, axis=-1, keepdims=True)
    p = jnp.exp2((s - m) * (scale * _LOG2E))
    l = jnp.sum(p, axis=-1, keepdims=True)
    o = jnp.dot(p.astype(v.dtype), v, preferred_element_type=jnp.float32)
    return o * (1.0 / l)


@jax.jit
def pallas_standalone__mha_softmax__near_ridge_kernel(
    q: jax.Array,
    k: jax.Array,
    v: jax.Array,
):
    B, H, S, D = q.shape
    assert k.shape == q.shape and v.shape == q.shape
    assert k.dtype == q.dtype and v.dtype == q.dtype
    N = B * H
    scale = D ** -0.5

    c = 4
    R = 4
    n = N // c
    rows = 64
    pph = S // rows
    P = c * pph
    total_rows = N * S
    nw = total_rows // rows
    Rw = 16
    G = 4
    rounds = nw // Rw
    tail_heads = R * c
    assert N % c == 0 and n >= R and S % rows == 0
    assert Rw % G == 0 and nw % Rw == 0 and tail_heads < rounds - 1
    assert tail_heads + 1 <= rounds - (tail_heads * pph * G + Rw - 1) // Rw

    def kernel_function(q_h, k_h, v_h, o_h, buf, obuf, rsem, wsem):
        hb = (q_h, k_h, v_h)

        def read_start(i, slot):
            u = 0
            for p in range(P):
                for s in range(3):
                    pltpu.make_async_copy(
                        hb[s].at[i * P + p], buf.at[slot, s, p], rsem.at[slot]
                    ).start(priority=u % 2)
                    u += 1

        def read_wait(slot):
            pltpu.make_async_copy(buf.at[slot], buf.at[slot], rsem.at[slot]).wait()

        def write(rho, w):
            r = ((w % G) * (nw // G) + w // G) * rows + rho * (Rw // G * rows)
            if not isinstance(r, int):
                r = pl.multiple_of(r, rows)
            return pltpu.make_async_copy(
                obuf.at[pl.ds(r, rows)], o_h.at[pl.ds(r, rows)], wsem.at[w]
            )

        def compute(i, slot, u):
            def load(s):
                return buf[slot, s, pl.ds(u * pph, pph)].reshape(S, D)

            r = pl.multiple_of((i * c + u) * S, S)
            obuf[pl.ds(r, S), :] = _attend(load(0), load(1), load(2), scale).astype(
                obuf.dtype
            )

        for i in range(R):
            read_start(i, i)

        def read_body(i, carry):
            slot = i % R
            read_wait(slot)
            for u in range(c):
                compute(i, slot, u)
            read_start(i + R, slot)
            return carry

        jax.lax.fori_loop(0, n - R, read_body, None)

        for i in range(n - R, n):
            read_wait(i % R)
        for w in range(Rw):
            write(0, w).start()

        def service(rho):
            for w in range(Rw):
                write(rho, w).wait()
                write(rho + 1, w).start()

        def tail_body(rho, carry):
            i = n - R + rho // c
            compute(i, i % R, rho % c)
            service(rho)
            return carry

        jax.lax.fori_loop(0, tail_heads, tail_body, None)

        def write_body(rho, carry):
            service(rho)
            return carry

        jax.lax.fori_loop(tail_heads, rounds - 1, write_body, None)
        for w in range(Rw):
            write(rounds - 1, w).wait()

    out = pl.pallas_call(
        kernel_function,
        in_specs=[pl.BlockSpec(memory_space=pl.ANY)] * 3,
        out_specs=pl.BlockSpec(memory_space=pl.ANY),
        out_shape=jax.ShapeDtypeStruct((total_rows, D), v.dtype),
        scratch_shapes=[
            pltpu.VMEM((R, 3, P, rows, D), q.dtype),
            pltpu.VMEM((total_rows, D), v.dtype),
            pltpu.SemaphoreType.DMA((R,)),
            pltpu.SemaphoreType.DMA((Rw,)),
        ],
        compiler_params=pltpu.CompilerParams(
            vmem_limit_bytes=64 * 1024 * 1024, disable_bounds_checks=True
        ),
    )(
        q.reshape(total_rows // rows, rows, D),
        k.reshape(total_rows // rows, rows, D),
        v.reshape(total_rows // rows, rows, D),
    )
    return out.reshape(B, H, S, D)
```

```python
import math

import jax
import jax.numpy as jnp
import jax.experimental.pallas as pl
import jax.experimental.pallas.tpu as pltpu

_LOG2E = math.log2(math.e)


def _attend(q, k, v, scale):
    s = jax.lax.dot_general(
        q, k, (((1,), (1,)), ((), ())), preferred_element_type=jnp.float32
    )
    m = jnp.max(s, axis=-1, keepdims=True)
    p = jnp.exp2((s - m) * (scale * _LOG2E))
    l = jnp.sum(p, axis=-1, keepdims=True)
    o = jnp.dot(p.astype(v.dtype), v, preferred_element_type=jnp.float32)
    return o * (1.0 / l)


@jax.jit
def pallas_standalone__mha_softmax__near_ridge_kernel(
    q: jax.Array,
    k: jax.Array,
    v: jax.Array,
):
    B, H, S, D = q.shape
    assert k.shape == q.shape and v.shape == q.shape
    assert k.dtype == q.dtype and v.dtype == q.dtype
    N = B * H
    scale = D ** -0.5

    c = 4
    n = N // c
    R = 4
    rows = 64
    pph = S // rows
    pa = pph - 1
    total_rows = N * S
    nw = total_rows // rows
    Rw = 16
    G = 8
    rounds = nw // Rw
    tail_heads = R * c
    assert N % c == 0 and n >= R and S % rows == 0 and pph >= 2
    assert Rw % G == 0 and nw % Rw == 0 and (nw // G) % pph == 0
    assert G % c == 0 and R <= N // G
    deferred_rounds = -(-R * pph // (Rw // G))
    assert tail_heads <= rounds - deferred_rounds - 1

    def kernel_function(q_h, k_h, v_h, o_h, buf, obuf, rsem, wsem):
        hb = (q_h, k_h, v_h)

        def read_start(i, slot):
            j = 0
            for p in range(pph):
                for s in range(3):
                    for u in range(c):
                        pltpu.make_async_copy(
                            hb[s].at[(u * n + i) * pph + p],
                            buf.at[slot, p, s, u],
                            rsem.at[slot, int(p >= pa)],
                        ).start(priority=j % 2)
                        j += 1

        def read_wait(slot, group):
            view = buf.at[slot, pl.ds(0, pa)] if group == 0 else buf.at[slot, pl.ds(pa, 1)]
            pltpu.make_async_copy(view, view, rsem.at[slot, group]).wait()

        def write(rho, w):
            r = ((w % G) * (nw // G) + w // G) * rows + rho * (Rw // G * rows)
            if not isinstance(r, int):
                r = pl.multiple_of(r, rows)
            return pltpu.make_async_copy(
                obuf.at[pl.ds(r, rows)], o_h.at[pl.ds(r, rows)], wsem.at[w]
            )

        def compute(i, slot, u):
            def load(s):
                return buf[slot, :, s, u].reshape(S, D)

            r = pl.multiple_of((u * n + i) * S, S)
            obuf[pl.ds(r, S), :] = _attend(load(0), load(1), load(2), scale).astype(
                obuf.dtype
            )

        for i in range(R):
            read_start(i, i)

        def read_body(i, carry):
            slot = i % R
            read_wait(slot, 0)
            read_wait(slot, 1)
            for u in range(c):
                compute(i, slot, u)
            read_start(i + R, slot)
            return carry

        jax.lax.fori_loop(0, n - R, read_body, None)

        for i in range(n - R, n):
            read_wait(i % R, 0)
            if i < n - 1:
                read_wait(i % R, 1)
        for w in range(Rw):
            write(0, w).start()
        read_wait((n - 1) % R, 1)

        def service(rho, two_queues):
            for w in range(Rw):
                write(rho, w).wait()
                write(rho + 1, w).start(priority=w % 2 if two_queues else 0)

        def tail_body(rho, carry):
            i = n - R + rho // c
            compute(i, i % R, rho % c)
            service(rho, False)
            return carry

        jax.lax.fori_loop(0, tail_heads, tail_body, None)

        def write_body(rho, carry):
            service(rho, True)
            return carry

        jax.lax.fori_loop(tail_heads, rounds - 1, write_body, None)
        for w in range(Rw):
            write(rounds - 1, w).wait()

    out = pl.pallas_call(
        kernel_function,
        in_specs=[pl.BlockSpec(memory_space=pl.ANY)] * 3,
        out_specs=pl.BlockSpec(memory_space=pl.ANY),
        out_shape=jax.ShapeDtypeStruct((total_rows, D), v.dtype),
        scratch_shapes=[
            pltpu.VMEM((R, pph, 3, c, rows, D), q.dtype),
            pltpu.VMEM((total_rows, D), v.dtype),
            pltpu.SemaphoreType.DMA((R, 2)),
            pltpu.SemaphoreType.DMA((Rw,)),
        ],
        compiler_params=pltpu.CompilerParams(vmem_limit_bytes=64 * 1024 * 1024),
    )(
        q.reshape(total_rows // rows, rows, D),
        k.reshape(total_rows // rows, rows, D),
        v.reshape(total_rows // rows, rows, D),
    )
    return out.reshape(B, H, S, D)
```

```python
import math

import jax
import jax.numpy as jnp
import jax.experimental.pallas as pl
import jax.experimental.pallas.tpu as pltpu

_LOG2E = math.log2(math.e)


def _attend(q, k, v, scale):
    s = jax.lax.dot_general(
        q, k, (((1,), (1,)), ((), ())), preferred_element_type=jnp.float32
    )
    m = jnp.max(s, axis=-1, keepdims=True)
    p = jnp.exp2((s - m) * (scale * _LOG2E))
    l = jnp.sum(p, axis=-1, keepdims=True)
    o = jnp.dot(p.astype(v.dtype), v, preferred_element_type=jnp.float32)
    return o * (1.0 / l)


@jax.jit
def pallas_standalone__mha_softmax__near_ridge_kernel(
    q: jax.Array,
    k: jax.Array,
    v: jax.Array,
):
    B, H, S, D = q.shape
    assert k.shape == q.shape and v.shape == q.shape
    assert k.dtype == q.dtype and v.dtype == q.dtype
    N = B * H
    scale = D ** -0.5

    c = 4
    n = N // c
    R = 3
    rows = 64
    pph = S // rows
    pa = pph - 1
    total_rows = N * S
    G = 8
    hpr = N // G
    ppr = hpr * pph
    ppb = 8
    nbt = ppr // ppb
    NB = 2
    assert N % c == 0 and n >= R and S % rows == 0 and pph >= 2
    assert N % G == 0 and ppr % ppb == 0
    assert G % c == 0 and R <= hpr
    deferred = -(-R * pph // ppb)
    assert R - 1 + NB < nbt - deferred

    def kernel_function(q_h, k_h, v_h, o_h, buf, obuf, rsem, wsem):
        hb = (q_h, k_h, v_h)

        def read_start(i, slot):
            j = 0
            for p in range(pph):
                for s in range(3):
                    for u in range(c):
                        pltpu.make_async_copy(
                            hb[s].at[(u * n + i) * pph + p],
                            buf.at[slot, p, s, u],
                            rsem.at[slot, int(p >= pa)],
                        ).start(priority=j % 2)
                        j += 1

        def read_wait(slot, group):
            view = buf.at[slot, pl.ds(0, pa)] if group == 0 else buf.at[slot, pl.ds(pa, 1)]
            pltpu.make_async_copy(view, view, rsem.at[slot, group]).wait()

        def write_start(b, slot):
            for p in range(ppb):
                for g in range(G):
                    pltpu.make_async_copy(
                        obuf.at[g, b * ppb + p], o_h.at[g, b * ppb + p], wsem.at[slot]
                    ).start(priority=g % 2)

        def write_wait(b, slot):
            pltpu.make_async_copy(
                obuf.at[:, pl.ds(b * ppb, ppb)],
                o_h.at[:, pl.ds(b * ppb, ppb)],
                wsem.at[slot],
            ).wait()

        def compute(i, slot, u):
            def load(s):
                return buf[slot, :, s, u].reshape(S, D)

            h = u * n + i
            o = _attend(load(0), load(1), load(2), scale).astype(obuf.dtype)
            obuf[h // hpr, pl.ds((h % hpr) * pph, pph)] = o.reshape(pph, rows, D)

        for i in range(R):
            read_start(i, i)

        def read_body(i, carry):
            slot = i % R
            read_wait(slot, 0)
            read_wait(slot, 1)
            for u in range(c):
                compute(i, slot, u)
            read_start(i + R, slot)
            return carry

        jax.lax.fori_loop(0, n - R, read_body, None)

        for i in range(n - R, n):
            read_wait(i % R, 0)
            if i < n - 1:
                read_wait(i % R, 1)
        for b in range(NB):
            write_start(b, b)
        read_wait((n - 1) % R, 1)

        def tail_body(b, carry):
            i = n - R + b
            for u in range(c):
                compute(i, i % R, u)
            write_wait(b, b % NB)
            write_start(b + NB, b % NB)
            return carry

        jax.lax.fori_loop(0, R, tail_body, None)

        def write_body(b, carry):
            write_wait(b, b % NB)
            write_start(b + NB, b % NB)
            return carry

        jax.lax.fori_loop(R, nbt - NB, write_body, None)
        for b in range(nbt - NB, nbt):
            write_wait(b, b % NB)

    out = pl.pallas_call(
        kernel_function,
        in_specs=[pl.BlockSpec(memory_space=pl.ANY)] * 3,
        out_specs=pl.BlockSpec(memory_space=pl.ANY),
        out_shape=jax.ShapeDtypeStruct((G, ppr, rows, D), v.dtype),
        scratch_shapes=[
            pltpu.VMEM((R, pph, 3, c, rows, D), q.dtype),
            pltpu.VMEM((G, ppr, rows, D), v.dtype),
            pltpu.SemaphoreType.DMA((R, 2)),
            pltpu.SemaphoreType.DMA((NB,)),
        ],
        compiler_params=pltpu.CompilerParams(vmem_limit_bytes=64 * 1024 * 1024),
    )(
        q.reshape(total_rows // rows, rows, D),
        k.reshape(total_rows // rows, rows, D),
        v.reshape(total_rows // rows, rows, D),
    )
    return out.reshape(B, H, S, D)
```
